```python
import os as _os
_os.environ.setdefault("JAX_PLATFORMS", "cpu")
import jax
import jax.numpy as jnp

def _softmax(x, axis=-1):
    return jax.nn.softmax(x, axis=axis)
def _gelu(x):
    return jax.nn.gelu(x, approximate=True)
def _silu(x):
    return jax.nn.silu(x)
def _sigmoid(x):
    return jax.nn.sigmoid(x)
def _layernorm(x, axis=-1, eps=1e-5):
    m = jnp.mean(x, axis=axis, keepdims=True)
    v = jnp.var(x, axis=axis, keepdims=True)
    return (x - m) / jnp.sqrt(v + eps)
def _scatter_add(tgt, idx, src, axis=0):
    return tgt.at[idx].add(src)
def _segment_sum(src, seg, n):
    return jax.ops.segment_sum(src, seg, n)
class _Rng:
    def __init__(self, key):
        self._k = key
    def _next(self):
        self._k, sub = jax.random.split(self._k)
        return sub
    def normal(self, shape):
        return jax.random.normal(self._next(), shape, dtype=jnp.bfloat16)
    def randint(self, lo, hi, shape):
        return jax.random.randint(self._next(), shape, lo, hi, dtype=jnp.int32)
    def uniform(self, shape, lo=0.0, hi=1.0):
        return jax.random.uniform(self._next(), shape, jnp.bfloat16, lo, hi)
    def permutation(self, n):
        return jax.random.permutation(self._next(), n)


kernel_name = 'standalone__linear_kernel_hedgehog__prompt'

def setup_inputs():
    _rng = _Rng(jax.random.key(int.from_bytes(__import__("os").urandom(4), "little")))
    _w = (lambda a: (lambda t: t.astype(jnp.bfloat16) if jnp.issubdtype(t.dtype, jnp.floating) else t)(jnp.asarray(a)))
    B, S, D, H = 1, 2048, 1024, 32
    Dh = D // H
    return {
        "x": _w((lambda *s: _rng.normal(s) * 0.4)(B, S, D)),
        "wqkv": _w((lambda *s: _rng.normal(s) * 0.4)(D, 3 * D)),
        "w_phi": _w((lambda *s: _rng.normal(s) * 0.4)(H, Dh, Dh) * (Dh ** -0.5)),
        "wo": _w((lambda *s: _rng.normal(s) * 0.05)(D, D)),
    }

def reference(x, wqkv, w_phi, wo):
    B, S, D = x.shape
    H = 32; Dh = D // H
    qkv = (lambda x, *d: x.transpose(*d))((x @ wqkv).reshape(B, S, 3, H, Dh), 2, 0, 3, 1, 4)
    q, k, v = qkv[0], qkv[1], qkv[2]
    pq = jnp.einsum("bhsd,hdf->bhsf", q, w_phi)
    pk = jnp.einsum("bhsd,hdf->bhsf", k, w_phi)
    phi_q = jnp.concatenate([_softmax(pq, axis=-1), _softmax(-pq, axis=-1)], axis=-1)
    phi_k = jnp.concatenate([_softmax(pk, axis=-1), _softmax(-pk, axis=-1)], axis=-1)
    kv = jnp.einsum("bhsf,bhsd->bhfd", phi_k, v)
    z  = jnp.einsum("bhsf->bhf", phi_k)
    num = jnp.einsum("bhqf,bhfd->bhqd", phi_q, kv)
    den = jnp.einsum("bhqf,bhf->bhq", phi_q, z)[..., None] + 1e-6
    o = num / den
    return (lambda x, *d: x.transpose(*d))(o, 0, 2, 1, 3).reshape(B, S, D) @ wo
```

```python
import contextlib
import numpy as np
import jax
import jax.numpy as jnp
from jax import lax
from jax.experimental import pallas as pl
from jax.experimental.pallas import tpu as pltpu

LOG2E = 1.4426950408889634
NT = (((1,), (1,)), ((), ()))
f32 = jnp.float32
bf16 = jnp.bfloat16
u32 = jnp.uint32


def mo(v, m):
    return v if isinstance(v, int) else pl.multiple_of(v, m)


def make_kernel(TS=512, S=2048, D=1024, H=32, nodma_in=False, nodma_out=False, flags=None,
                rcp="nr", scopes=False, nobc=False, RB=16, midmode=0, PB=64):
    class _N:
        def start(self): pass
        def wait(self): pass
    mk_in = (lambda *a: _N()) if nodma_in else pltpu.make_async_copy
    mk_out = (lambda *a: _N()) if nodma_out else pltpu.make_async_copy
    NC = S // TS
    assert NC == 4
    Dh = 32
    NP = H // 2
    TH = TS // 2
    DH = D // 2

    def recip(x):
        if rcp == "div":
            return 1.0 / x
        if rcp == "nr":
            return pltpu.reciprocal(x, approx=False, full_range=False)
        return pltpu.reciprocal(x, approx=True)

    def kernel(x_hbm, w_hbm, wphi_hbm, wo_hbm, o_hbm,
               x_v, w_v, wo_v, wphi_v, out_v,
               ws_u, xs_u, wos_u, bd_u, vt_u, phik_u, phiq_u, ot_u,
               kvz_v, o32_v,
               sem_x, sem_wk, sem_w, sem_small, sem_o):
        ws = ws_u.bitcast(bf16)
        xs = xs_u.bitcast(bf16)
        wos = wos_u.bitcast(bf16)
        bd = bd_u.bitcast(bf16)
        vt = vt_u.bitcast(bf16)
        phik = phik_u.bitcast(bf16)
        phiq = phiq_u.bitcast(bf16)
        ot = ot_u.bitcast(bf16)
        sc = (lambda n: jax.named_scope(n)) if scopes else (lambda n: contextlib.nullcontext())

        def cp_x(c):
            return mk_in(x_hbm.at[pl.ds(mo(c * TS, TS), TS), :], x_v.at[pl.ds(mo(c * TS, TS), TS), :], sem_x.at[c])

        def cp_wk(j, half):
            r0 = j * 128 + half * DH
            return mk_in(w_hbm.at[pl.ds(r0, 128), pl.ds(D, D)], w_v.at[pl.ds(r0, 128), pl.ds(D, D)], sem_wk.at[j, half])

        def cp_w(t):
            return mk_in(w_hbm.at[:, pl.ds(t * D, D)], w_v.at[:, pl.ds(t * D, D)], sem_w.at[t])

        cp_phi = mk_in(wphi_hbm, wphi_v, sem_small.at[0])
        cp_wo = mk_in(wo_hbm, wo_v, sem_small.at[1])

        def cp_out(c, k):
            if k == 0:
                r0, c0, nc = c * TS + TH, 0, DH
            elif k == 1:
                r0, c0, nc = c * TS, 0, D
            else:
                r0, c0, nc = c * TS + TH, DH, DH
            r0 = mo(r0, TH)
            return mk_out(out_v.at[pl.ds(r0, TH), pl.ds(c0, nc)], o_hbm.at[pl.ds(r0, TH), pl.ds(c0, nc)], sem_o.at[c, k])

        cp_phi.start()
        for j in range(4):
            for h in range(2):
                cp_wk(j, h).start()
        cp_x(0).start()

        for p in range(NP):
            vt.at[p][64:80, :] = jnp.ones((16, TS), bf16)
        kvz_v[...] = jnp.zeros(kvz_v.shape, f32)

        cp_phi.wait()
        cp_w(2).start()
        r = lax.broadcasted_iota(jnp.int32, (128, 128), 0)
        c_ = lax.broadcasted_iota(jnp.int32, (128, 128), 1)
        eye32 = (lax.broadcasted_iota(jnp.int32, (128, Dh), 0) % Dh == lax.broadcasted_iota(jnp.int32, (128, Dh), 1)).astype(bf16)
        mask_bd = (r // 32) == (c_ // 32)
        for g in range(8):
            w4 = wphi_v[pl.ds(g * 128, 128), :]
            t = lax.dot_general(eye32, w4, NT, preferred_element_type=f32)
            bd[:, pl.ds(g * 128, 128)] = jnp.where(mask_bd, t, 0.0).astype(bf16)

        def a_ops(a11, a12, a21, a22):
            return [a11 + a22, a21 + a22, a11, a22, a11 + a12, a21 - a11, a12 - a22]

        def b_ops(b11, b12, b21, b22):
            return [b11 + b22, b11, b12 - b22, b21 - b11, b22, b11 + b12, b21 + b22]

        def store_wsums(slot, g, c0, ncol, a11, a12, a21, a22):
            for r0 in range(0, 128, RB):
                ops = a_ops(a11[r0:r0 + RB], a12[r0:r0 + RB], a21[r0:r0 + RB], a22[r0:r0 + RB])
                for i in range(7):
                    ws.at[slot, i][pl.ds(g * 128 + r0, RB), pl.ds(c0, ncol)] = ops[i].astype(bf16)

        def fold_block(t, slot, j, ncol=128):
            for g in range(4):
                def one(gg, r0):
                    blk = w_v[pl.ds(r0, ncol), pl.ds(t * D + gg * 128, 128)]
                    return lax.dot_general(bd[:, pl.ds(gg * 128, 128)], blk, NT, preferred_element_type=f32) * LOG2E
                store_wsums(slot, g, j * ncol, ncol, one(g, j * ncol), one(g, DH + j * ncol), one(g + 4, j * ncol), one(g + 4, DH + j * ncol))

        def vprep_block(slot, j, ncol=128):
            for g in range(4):
                def one(gg, r0):
                    blk = w_v[pl.ds(r0, ncol), pl.ds(2 * D + gg * 128, 128)]
                    return blk.T
                q = [one(g, j * ncol), one(g, DH + j * ncol), one(g + 4, j * ncol), one(g + 4, DH + j * ncol)]
                for r0 in range(0, 128, RB):
                    ops = a_ops(*[v[r0:r0 + RB].astype(f32) for v in q])
                    for i in range(7):
                        ws.at[slot, i][pl.ds(g * 128 + r0, RB), pl.ds(j * ncol, ncol)] = ops[i].astype(bf16)

        def prep_x(c):
            for r0 in range(0, TH, RB):
                ra = mo(c * TS + r0, RB)
                rb = mo(c * TS + TH + r0, RB)
                b11 = x_v[pl.ds(ra, RB), :DH].astype(f32)
                b21 = x_v[pl.ds(ra, RB), DH:].astype(f32)
                b12 = x_v[pl.ds(rb, RB), :DH].astype(f32)
                b22 = x_v[pl.ds(rb, RB), DH:].astype(f32)
                ops = b_ops(b11, b12, b21, b22)
                for i in (1, 4, 0, 2, 5, 3, 6):
                    xs.at[c, i][pl.ds(r0, RB), :] = ops[i].astype(bf16)

        def prep_wo(j):
            for r0 in range(0, 128, RB):
                q0 = mo(j * 128 + r0, RB)
                q1 = mo(j * 128 + DH + r0, RB)
                b11 = wo_v[pl.ds(q0, RB), :DH].astype(f32)
                b12 = wo_v[pl.ds(q0, RB), DH:].astype(f32)
                b21 = wo_v[pl.ds(q1, RB), :DH].astype(f32)
                b22 = wo_v[pl.ds(q1, RB), DH:].astype(f32)
                ops = b_ops(b11, b12, b21, b22)
                for i in range(7):
                    wos.at[i][pl.ds(q0, RB), :] = ops[i].astype(bf16)

        def softmax_head(p, dst, hh, tok0):
            mx = jnp.max(p, axis=0, keepdims=True)
            mn = jnp.min(p, axis=0, keepdims=True)
            e1 = jnp.exp2(p - mx)
            e2 = jnp.exp2(mn - p)
            r1 = recip(jnp.sum(e1, axis=0, keepdims=True))
            r2 = recip(jnp.sum(e2, axis=0, keepdims=True))
            dst[pl.ds(hh * 64, 32), pl.ds(tok0, TH)] = (e1 * r1).astype(bf16)
            dst[pl.ds(hh * 64 + 32, 32), pl.ds(tok0, TH)] = (e2 * r2).astype(bf16)

        def softmax_block(terms, dst, head0, tok0):
            for h in range(16):
                sl = slice(h * 32, (h + 1) * 32)
                p = terms[0][1][sl]
                for sg, t in terms[1:]:
                    p = p + t[sl] if sg > 0 else p - t[sl]
                softmax_head(p, dst, head0 + h, tok0)

        def comb(terms, sl):
            p = terms[0][1][sl]
            for sg, t in terms[1:]:
                p = p + t[sl] if sg > 0 else p - t[sl]
            return p

        def prod(slot, c):
            return lambda i: lax.dot_general(ws.at[slot, i - 1][...], xs.at[c, i - 1][...], NT, preferred_element_type=f32)

        with sc("prologue"):
            for j in range(4):
                cp_wk(j, 0).wait()
                cp_wk(j, 1).wait()
                fold_block(1, 0, j)

        def body1a(c, carry):
            cp_x(c).wait()

            @pl.when(c + 1 < NC)
            def _():
                cp_x(c + 1).start()

            @pl.when(c == 0)
            def _():
                cp_w(0).start()

            @pl.when(c == 1)
            def _():
                cp_wo.start()
            prep_x(c)
            m = prod(0, c)
            dst = phik.at[c]
            m2 = m(2)
            m5 = m(5)
            m1 = m(1)
            m3 = m(3)
            softmax_block([(1, m3), (1, m5)], dst, 0, TH)
            m6 = m(6)
            softmax_block([(1, m1), (-1, m2), (1, m3), (1, m6)], dst, 16, TH)
            m4 = m(4)
            softmax_block([(1, m2), (1, m4)], dst, 16, 0)
            m7 = m(7)
            softmax_block([(1, m1), (1, m4), (-1, m5), (1, m7)], dst, 0, 0)
            return carry

        def body1b(c, carry):
            m = prod(1, c)

            def put(terms, p0, t0):
                for p in range(NP // 2):
                    for r0 in range(0, 64, 16):
                        vt.at[p0 + p][r0:r0 + 16, t0:t0 + TH] = comb(terms, slice(p * 64 + r0, p * 64 + r0 + 16)).astype(bf16)
            m2 = m(2)
            m1 = m(1)
            m3 = m(3)
            m6 = m(6)
            put([(1, m1), (-1, m2), (1, m3), (1, m6)], 8, TH)
            m4 = m(4)
            put([(1, m2), (1, m4)], 8, 0)
            m5 = m(5)
            put([(1, m3), (1, m5)], 0, TH)
            m7 = m(7)
            put([(1, m1), (1, m4), (-1, m5), (1, m7)], 0, 0)
            for p in list(range(8, 16)) + list(range(8)):
                kvz_v[p] += lax.dot_general(vt.at[p][...], phik.at[c][pl.ds(p * 128, 128), :], NT, preferred_element_type=f32)
            if midmode == 0:
                prep_wo(c)
            return carry

        rr = lax.broadcasted_iota(jnp.int32, (80, 128), 0)
        cc = lax.broadcasted_iota(jnp.int32, (80, 128), 1)
        row_head = jnp.where(rr < 64, rr // 32, (rr - 64) // 8)
        mk = row_head == (cc // 64)

        def body2(c, carry):
            m = prod(2, c)

            def nd_block(p0, t0):
                for p in range(p0, p0 + 8):
                    kvm = jnp.where(mk, kvz_v[p], 0.0).astype(bf16)
                    nd = jnp.dot(kvm, phiq[pl.ds(p * 128, 128), pl.ds(t0, TH)], preferred_element_type=f32)
                    rd = recip(nd[64:80] + 1e-6)
                    for hl in range(2):
                        rrep = jnp.concatenate([rd[hl * 8:hl * 8 + 8]] * 4, axis=0)
                        o32_v[pl.ds(p * 64 + hl * 32, 32), pl.ds(t0, TH)] = nd[hl * 32:hl * 32 + 32] * rrep

            def set_as(which):
                for r0 in range(0, DH, RB):
                    A11 = lambda: o32_v[r0:r0 + RB, 0:TH]
                    A12 = lambda: o32_v[DH + r0:DH + r0 + RB, 0:TH]
                    A21 = lambda: o32_v[r0:r0 + RB, TH:TS]
                    A22 = lambda: o32_v[DH + r0:DH + r0 + RB, TH:TS]
                    f = {1: lambda: A11() + A22(), 2: lambda: A21() + A22(), 3: A11, 4: A22,
                         5: lambda: A11() + A12(), 6: lambda: A21() - A11(), 7: lambda: A12() - A22()}
                    for i in which:
                        ot.at[i - 1][pl.ds(r0, RB), :] = f[i]().astype(bf16)

            def mo_(i):
                return jnp.dot(ot.at[i - 1][...].T, wos.at[i - 1][...], preferred_element_type=f32)

            def put_out(terms, r0, c0):
                for q in range(0, TH, RB):
                    out_v[pl.ds(mo(c * TS + r0 + q, RB), RB), c0:c0 + DH] = comb(terms, slice(q, q + RB)).astype(bf16)

            m2 = m(2)
            m1 = m(1)
            m3 = m(3)
            m6 = m(6)
            softmax_block([(1, m1), (-1, m2), (1, m3), (1, m6)], phiq, 16, TH)
            m4 = m(4)
            softmax_block([(1, m2), (1, m4)], phiq, 16, 0)
            nd_block(8, TH)
            m5 = m(5)
            softmax_block([(1, m3), (1, m5)], phiq, 0, TH)
            nd_block(8, 0)
            set_as([4])
            m7 = m(7)
            softmax_block([(1, m1), (1, m4), (-1, m5), (1, m7)], phiq, 0, 0)
            nd_block(0, TH)
            set_as([7])
            n4 = mo_(4)
            nd_block(0, 0)
            set_as([2])
            n7 = mo_(7)
            set_as([1, 3])
            n2 = mo_(2)
            put_out([(1, n2), (1, n4)], TH, 0)
            cp_out(c, 0).start()
            set_as([5, 6])
            n1 = mo_(1)
            n3 = mo_(3)
            n5 = mo_(5)
            put_out([(1, n3), (1, n5)], 0, DH)
            put_out([(1, n1), (1, n4), (-1, n5), (1, n7)], 0, 0)
            cp_out(c, 1).start()
            n6 = mo_(6)
            put_out([(1, n1), (-1, n2), (1, n3), (1, n6)], TH, DH)
            cp_out(c, 2).start()
            return carry

        def run(body):
            lax.fori_loop(0, NC, body, 0)

        with sc("L1a"):
            run(body1a)
        with sc("mid1"):
            cp_w(2).wait()
            cp_w(0).wait()
            cp_wo.wait()
            for j in range(4):
                vprep_block(1, j)
                fold_block(0, 2, j)
                if midmode == 1:
                    prep_wo(j)
        with sc("L1b"):
            run(body1b)
        with sc("L2"):
            run(body2)
        with sc("tail"):
            for c in range(NC):
                for k in range(3):
                    cp_out(c, k).wait()

    def call(x, wqkv, w_phi, wo):
        x2 = x.reshape(S, D)
        wp = w_phi.reshape(H * Dh, Dh)
        out = pl.pallas_call(
            kernel,
            out_shape=jax.ShapeDtypeStruct((S, D), bf16),
            in_specs=[pl.BlockSpec(memory_space=pl.ANY)] * 4,
            out_specs=pl.BlockSpec(memory_space=pl.ANY),
            scratch_shapes=[
                pltpu.VMEM((S, D), bf16),
                pltpu.VMEM((D, 3 * D), bf16),
                pltpu.VMEM((D, D), bf16),
                pltpu.VMEM((H * Dh, Dh), bf16),
                pltpu.VMEM((S, D), bf16),
                pltpu.VMEM((3, 7, DH // 2, DH), u32),
                pltpu.VMEM((NC, 7, TH // 2, DH), u32),
                pltpu.VMEM((7, DH // 2, DH), u32),
                pltpu.VMEM((64, 1024), u32),
                pltpu.VMEM((NP, 40, TS), u32),
                pltpu.VMEM((NC, D, TS), u32),
                pltpu.VMEM((D, TS), u32),
                pltpu.VMEM((7, DH // 2, TH), u32),
                pltpu.VMEM((NP, 80, 128), f32),
                pltpu.VMEM((D, TS), f32),
                pltpu.SemaphoreType.DMA((NC,)),
                pltpu.SemaphoreType.DMA((4, 2)),
                pltpu.SemaphoreType.DMA((3,)),
                pltpu.SemaphoreType.DMA((2,)),
                pltpu.SemaphoreType.DMA((NC, 3)),
            ],
            compiler_params=pltpu.CompilerParams(vmem_limit_bytes=100 * 1024 * 1024, flags=flags, disable_bounds_checks=nobc),
        )(x2, wqkv, wp, wo)
        return out.reshape(1, S, D)

    return call


_CALL = make_kernel(nobc=True)


@jax.jit
def pallas_standalone__linear_kernel_hedgehog__prompt_kernel(
    x: jax.Array,
    wqkv: jax.Array,
    w_phi: jax.Array,
    wo: jax.Array,
):
    return _CALL(x, wqkv, w_phi, wo)
```

```python
import contextlib
import numpy as np
import jax
import jax.numpy as jnp
from jax import lax
from jax.experimental import pallas as pl
from jax.experimental.pallas import tpu as pltpu

LOG2E = 1.4426950408889634
NT = (((1,), (1,)), ((), ()))
f32 = jnp.float32
bf16 = jnp.bfloat16
u32 = jnp.uint32


def mo(v, m):
    return v if isinstance(v, int) else pl.multiple_of(v, m)


A_OPS = {1: [(1, (0, 0)), (1, (1, 1))], 2: [(1, (1, 0)), (1, (1, 1))], 3: [(1, (0, 0))], 4: [(1, (1, 1))],
         5: [(1, (0, 0)), (1, (0, 1))], 6: [(1, (1, 0)), (-1, (0, 0))], 7: [(1, (0, 1)), (-1, (1, 1))]}
B_OPS = {1: [(1, (0, 0)), (1, (1, 1))], 2: [(1, (0, 0))], 3: [(1, (0, 1)), (-1, (1, 1))], 4: [(1, (1, 0)), (-1, (0, 0))],
         5: [(1, (1, 1))], 6: [(1, (0, 0)), (1, (0, 1))], 7: [(1, (1, 0)), (1, (1, 1))]}
C_OPS = {(0, 0): [(1, 1), (1, 4), (-1, 5), (1, 7)], (0, 1): [(1, 3), (1, 5)],
         (1, 0): [(1, 2), (1, 4)], (1, 1): [(1, 1), (-1, 2), (1, 3), (1, 6)]}


def lincomb(terms):
    acc = terms[0][1]
    for sg, v in terms[1:]:
        acc = acc + v if sg > 0 else acc - v
    return acc


def completions(order):
    seen, out = set(), []
    for i in order:
        seen.add(i)
        out.append([q for q, t in C_OPS.items() if i in [k for _, k in t] and all(k in seen for _, k in t)])
    return out


class Tasks:
    def __init__(self, lag, budget):
        self.q, self.n, self.lag, self.budget = [], 0, lag, budget

    def add(self, key, fn):
        self.q.append((self.n, key, fn))

    def step(self):
        self.n += 1
        k = 0
        while self.q and k < self.budget and self.q[0][0] <= self.n - 1 - self.lag:
            self.q.pop(0)[2]()
            k += 1

    def flush(self, pred=None):
        rest = []
        for t in self.q:
            if pred is None or pred(t[1]):
                t[2]()
            else:
                rest.append(t)
        self.q = rest


def make_kernel(TS=512, S=2048, D=1024, H=32, nodma_in=False, nodma_out=False, flags=None,
                rcp="nr", scopes=False, nobc=True, RB=16, lk=2, lv=2, lq=2,
                ordA=(5, 3, 2, 4, 1, 7, 6), ordB=(5, 3, 2, 4, 1, 7, 6), ordC=(5, 3, 1, 4, 7, 2, 6),
                ordin=(5, 3, 2, 4, 1, 7, 6), lag=0, budget=1000, budget1=1000, pair=True, via=True, fb16=True, fstage=True, qpos=0):
    class _N:
        def start(self): pass
        def wait(self): pass
    mk_in = (lambda *a: _N()) if nodma_in else pltpu.make_async_copy
    mk_out = (lambda *a: _N()) if nodma_out else pltpu.make_async_copy
    NC = S // TS
    assert NC == 4
    Dh = 32
    NP = H // 2
    TH = TS // 2
    TQ = TS // 4
    DH = D // 2
    DQ = D // 4
    SK, SV, SQ = 0, 1, 2
    LV = {SK: lk, SV: lv, SQ: lq}
    X2 = 2 in LV.values()
    X1 = 1 in LV.values()

    def recip(x):
        if rcp == "div":
            return 1.0 / x
        if rcp == "nr":
            return pltpu.reciprocal(x, approx=False, full_range=False)
        return pltpu.reciprocal(x, approx=True)

    def kernel(x_hbm, w_hbm, wphi_hbm, wo_hbm, o_hbm,
               x_v, w_v, wo_v, wphi_v, out_v,
               wsk_u, wsv_u, wsq_u, xs1_u, xs2_u, wos_u, bd_u, vt_u, phi_u, ot_u,
               kvz_v, o32_v, pbuf_v, fst_u, flag_s,
               sem_x, sem_wv, sem_w, sem_small, sem_o):
        ws = [wsk_u.bitcast(bf16), wsv_u.bitcast(bf16), wsq_u.bitcast(bf16)]
        xs1 = xs1_u.bitcast(bf16)
        xs2 = xs2_u.bitcast(bf16)
        wos = wos_u.bitcast(bf16)
        bd = bd_u.bitcast(bf16)
        vt = vt_u.bitcast(bf16)
        phi = phi_u.bitcast(bf16)
        ot = ot_u.bitcast(bf16)
        fst = fst_u.bitcast(bf16)
        sc = (lambda n: jax.named_scope(n)) if scopes else (lambda n: contextlib.nullcontext())

        def cp_x(c):
            return mk_in(x_hbm.at[pl.ds(mo(c * TS, TS), TS), :], x_v.at[pl.ds(mo(c * TS, TS), TS), :], sem_x.at[c])

        def cp_wv(j):
            return mk_in(w_hbm.at[pl.ds(j * 128, 128), pl.ds(2 * D, D)], w_v.at[pl.ds(j * 128, 128), pl.ds(2 * D, D)], sem_wv.at[j])

        def cp_w(t):
            return mk_in(w_hbm.at[:, pl.ds(t * D, D)], w_v.at[:, pl.ds(t * D, D)], sem_w.at[t])

        cp_phi = mk_in(wphi_hbm, wphi_v, sem_small.at[0])
        cp_wo = mk_in(wo_hbm, wo_v, sem_small.at[1])

        def cp_out(c, k):
            if k == 0:
                r0, c0, nc = c * TS, DH, DH
            elif k == 1:
                r0, c0, nc = c * TS + TH, 0, D
            else:
                r0, c0, nc = c * TS, 0, DH
            r0 = mo(r0, TH)
            return mk_out(out_v.at[pl.ds(r0, TH), pl.ds(c0, nc)], o_hbm.at[pl.ds(r0, TH), pl.ds(c0, nc)], sem_o.at[c, k])

        wv_batches = [(0, 2, 4, 6), (1, 3, 5, 7)] if lv == 2 else [(0, 4), (1, 5), (2, 6), (3, 7)]
        for b in wv_batches:
            for j in b:
                cp_wv(j).start()
        cp_x(0).start()

        for c in range(NC):
            for p in range(NP):
                vt.at[c, p][64:80, :] = jnp.ones((16, TS), bf16)
        kvz_v[...] = jnp.zeros(kvz_v.shape, f32)

        def build_bd():
            r = lax.broadcasted_iota(jnp.int32, (128, 128), 0)
            c_ = lax.broadcasted_iota(jnp.int32, (128, 128), 1)
            r2 = lax.broadcasted_iota(jnp.int32, (128, Dh), 0)
            if pair:
                eye32 = (((r2 % 64) // 8) * 4 + (r2 % 8) // 2 == lax.broadcasted_iota(jnp.int32, (128, Dh), 1)).astype(bf16)
                mask_bd = ((r // 64) * 2 + r % 2) == (c_ // 32)
            else:
                eye32 = (r2 % Dh == lax.broadcasted_iota(jnp.int32, (128, Dh), 1)).astype(bf16)
                mask_bd = (r // 32) == (c_ // 32)
            for g in range(8):
                w4 = wphi_v[pl.ds(g * 128, 128), :]
                t = lax.dot_general(eye32, w4, NT, preferred_element_type=f32)
                bd[:, pl.ds(g * 128, 128)] = jnp.where(mask_bd, t, 0.0).astype(bf16)

        def ops1(table, q):
            return {i: lincomb([(sg, q[k]) for sg, k in t]) for i, t in table.items()}

        def ops2(table, blk):
            out = {}
            for i in table:
                sub = {(a, b): lincomb([(sg, blk[(2 * k[0] + a, 2 * k[1] + b)]) for sg, k in table[i]])
                       for a in range(2) for b in range(2)}
                for j, v in ops1(table, sub).items():
                    out[(i, j)] = v
            return out

        def w_tile(t, gg, j, lvl=1):
            blk = w_v[pl.ds(mo(j * 128, 128), 128), pl.ds(mo(t * D + gg * 128, 128), 128)]
            if t == 2:
                return blk.T
            res = lax.dot_general(bd[:, pl.ds(mo(gg * 128, 128), 128)], blk, NT, preferred_element_type=f32) * LOG2E
            return res.astype(bf16) if (fb16 and lvl == 2) else res

        def prep_w_l1(t, slot, j):
            for g in range(4):
                q = {(I, K): w_tile(t, g + 4 * I, j + 4 * K) for I in range(2) for K in range(2)}
                for r0 in range(0, 128, RB):
                    o = ops1(A_OPS, {k: v[r0:r0 + RB].astype(f32) for k, v in q.items()})
                    for i in range(1, 8):
                        ws[slot].at[i - 1][pl.ds(g * 128 + r0, RB), pl.ds(mo(j * 128, 128), 128)] = o[i].astype(bf16)

        def prep_w_l2(t, slot, u, w, dyn=None):
            q = {(R, K): w_tile(t, 2 * R + u, 2 * K + w, 2) for R in range(4) for K in range(4)}
            if fstage and dyn is not None:
                st = fst.at[lax.rem(dyn, 2)]
                ld = fst.at[dyn & 1]
                for (R, K), v in q.items():
                    st[pl.ds(R * 128, 128), pl.ds(K * 128, 128)] = v
                q = {(R, K): ld.at[pl.ds(R * 128, 128), pl.ds(K * 128, 128)] for (R, K) in q}
                if fstage == 2:
                    for r0 in range(0, 128, RB):
                        for i in range(1, 8):
                            sub = {(a, b): lincomb([(sg, q[(2 * k[0] + a, 2 * k[1] + b)][r0:r0 + RB].astype(f32)) for sg, k in A_OPS[i]])
                                   for a in range(2) for b in range(2)}
                            for j, v in ops1(A_OPS, sub).items():
                                ws[slot].at[(i - 1) * 7 + j - 1][pl.ds(mo(u * 128 + r0, RB), RB), pl.ds(mo(w * 128, 128), 128)] = v.astype(bf16)
                    return
            for r0 in range(0, 128, RB):
                o = ops2(A_OPS, {k: v[r0:r0 + RB].astype(f32) for k, v in q.items()})
                for (i, j), v in o.items():
                    ws[slot].at[(i - 1) * 7 + j - 1][pl.ds(mo(u * 128 + r0, RB), RB), pl.ds(mo(w * 128, 128), 128)] = v.astype(bf16)

        def prep_w_quarter(t, slot, part, dyn=None):
            if LV[slot] == 1:
                prep_w_l1(t, slot, part)
            else:
                prep_w_l2(t, slot, part // 2, part % 2, dyn)

        def prep_x1(c):
            for r0 in range(0, TH, RB):
                q = {(K, J): x_v[pl.ds(mo(c * TS + J * TH + r0, RB), RB), K * DH:(K + 1) * DH].astype(f32)
                     for K in range(2) for J in range(2)}
                o = ops1(B_OPS, q)
                for i in ordA:
                    xs1.at[c, i - 1][pl.ds(r0, RB), :] = o[i].astype(bf16)

        def prep_x2(c, i):
            for r0 in range(0, TQ, RB):
                def blk(K, J):
                    return x_v[pl.ds(mo(c * TS + J * TQ + r0, RB), RB), K * DQ:(K + 1) * DQ].astype(f32)
                sub = {(a, b): lincomb([(sg, blk(2 * k[0] + a, 2 * k[1] + b)) for sg, k in B_OPS[i]])
                       for a in range(2) for b in range(2)}
                o = ops1(B_OPS, sub)
                for j in ordin:
                    xs2.at[c, (i - 1) * 7 + j - 1][pl.ds(r0, RB), :] = o[j].astype(bf16)

        def prep_wo(j):
            for r0 in range(0, 128, RB):
                q = {(K, J): wo_v[pl.ds(mo(j * 128 + K * DH + r0, RB), RB), J * DH:(J + 1) * DH].astype(f32)
                     for K in range(2) for J in range(2)}
                o = ops1(B_OPS, q)
                for i in range(1, 8):
                    wos.at[i - 1][pl.ds(mo(j * 128 + r0, RB), RB), :] = o[i].astype(bf16)

        def softmax_head(p, dst, hh, tok0):
            n = p.shape[1]
            mx = jnp.max(p, axis=0, keepdims=True)
            mn = jnp.min(p, axis=0, keepdims=True)
            e1 = jnp.exp2(p - mx)
            e2 = jnp.exp2(mn - p)
            r1 = recip(jnp.sum(e1, axis=0, keepdims=True))
            r2 = recip(jnp.sum(e2, axis=0, keepdims=True))
            dst[pl.ds(hh * 64, 32), pl.ds(tok0, n)] = (e1 * r1).astype(bf16)
            dst[pl.ds(hh * 64 + 32, 32), pl.ds(tok0, n)] = (e2 * r2).astype(bf16)

        def allred(op, vs):
            while len(vs) > 1:
                vs = [op(vs[i], vs[i + 1]) for i in range(0, len(vs), 2)]
            v = vs[0]
            v = op(v, pltpu.roll(v, 4, 0))
            return op(v, pltpu.roll(v, 2, 0))

        def softmax_pair(p, dst, pp, tok0):
            n = p.shape[1]
            ps = [p[t * 8:(t + 1) * 8] for t in range(8)]
            mx = allred(jnp.maximum, ps)
            mn = allred(jnp.minimum, ps)
            e1 = [jnp.exp2(v - mx) for v in ps]
            e2 = [jnp.exp2(mn - v) for v in ps]
            r1 = recip(allred(jnp.add, e1))
            r2 = recip(allred(jnp.add, e2))
            for es, rcp_, off in ((e1, r1, 0), (e2, r2, 64)):
                for t in range(0, 8, 2):
                    dst[pl.ds(pp * 128 + off + t * 8, 16), pl.ds(tok0, n)] = \
                        jnp.concatenate([es[t] * rcp_, es[t + 1] * rcp_], axis=0).astype(bf16)

        SMR = 64 if pair else 32

        def softmax_rows(r0, t0, v):
            if pair:
                softmax_pair(v, phi, r0 // 64, t0)
            else:
                softmax_head(v, phi, r0 // 32, t0)

        def pmatmul(slot, c, order, SL, consume, tasks, before=None, after=None, bounce=False):
            if bounce:
                pst = pbuf_v.at[lax.rem(c, 2)]
                pld = pbuf_v.at[c & 1]
                consume0 = consume
                tasks0 = tasks

                class _T:
                    def add(self, key, fn):
                        self.key = key
                        fn()

                    def step(self):
                        tasks0.step()
                tasks = _T()

                def consume(r0, t0, v):
                    pst[pl.ds(r0, v.shape[0]), pl.ds(t0, v.shape[1])] = v
                    tasks0.add(tasks.key, lambda: consume0(r0, t0, pld[pl.ds(r0, v.shape[0]), pl.ds(t0, v.shape[1])]))
            if LV[slot] == 1:
                m = {}
                for n, (i, done) in enumerate(zip(order, completions(order))):
                    if before: before(n, i)
                    m[i] = lax.dot_general(ws[slot].at[i - 1][...], xs1.at[c, i - 1][...], NT, preferred_element_type=f32)
                    for (I, J) in done:
                        for r0 in range(0, DH, SL):
                            tasks.add((I, J), lambda I=I, J=J, r0=r0: consume(
                                I * DH + r0, J * TH, lincomb([(sg, m[k][r0:r0 + SL]) for sg, k in C_OPS[(I, J)]])))
                    tasks.step()
                    if after: after(n, i)
                return
            M = {}
            mm = {}

            def getM(i, a, b, r0):
                if (i, a, b, r0) not in M:
                    M[(i, a, b, r0)] = lincomb([(sg, mm[(i, kk)][r0:r0 + SL]) for sg, kk in C_OPS[(a, b)]])
                return M[(i, a, b, r0)]
            for n, (i, done) in enumerate(zip(order, completions(order))):
                if before: before(n, i)
                for j, done_in in zip(ordin, completions(ordin)):
                    k = (i - 1) * 7 + j - 1
                    mm[(i, j)] = lax.dot_general(ws[slot].at[k][...], xs2.at[c, k][...], NT, preferred_element_type=f32)
                    for (a, b) in done_in:
                        for r0 in range(0, DQ, SL):
                            if not done:
                                getM(i, a, b, r0)
                            for (I, J) in done:
                                tasks.add((I, J), lambda I=I, J=J, a=a, b=b, r0=r0: consume(
                                    (2 * I + a) * DQ + r0, (2 * J + b) * TQ,
                                    lincomb([(sg, getM(kk, a, b, r0)) for sg, kk in C_OPS[(I, J)]])))
                    tasks.step()
                if after: after(n, i)

        def mk_tasks(slot, scale):
            if LV[slot] == 1:
                return Tasks(0, budget1 * scale)
            return Tasks(lag, budget * scale)

        with sc("prologue"):
            for n, b in enumerate(wv_batches):
                for j in b:
                    cp_wv(j).wait()
                if n == 0:
                    cp_phi.start()
                    cp_w(1).start()
                if lv == 1:
                    prep_w_l1(2, SV, n)
                else:
                    for u in range(2):
                        prep_w_l2(2, SV, u, n)

        def bodyA(c, carry):
            cp_x(c).wait()

            @pl.when(c + 1 < NC)
            def _():
                cp_x(c + 1).start()

            @pl.when(c == 1)
            def _():
                cp_w(0).start()

            @pl.when(c == 2)
            def _():
                cp_wo.start()
            if lv == 1:
                prep_x1(c)
                if X2:
                    for i in range(1, 8):
                        prep_x2(c, i)
            else:
                for i in ordA:
                    prep_x2(c, i)
                if X1:
                    prep_x1(c)

            def put(r0, t0, v):
                vt.at[c, r0 // 64][pl.ds(r0 % 64, v.shape[0]), pl.ds(t0, v.shape[1])] = v.astype(bf16)
            tasks = mk_tasks(SV, 4)
            pmatmul(SV, c, ordA, 16, put, tasks)
            tasks.flush()
            return carry

        def bodyB(c, carry):
            tasks = mk_tasks(SK, 1)
            comp = completions(ordB)

            def kvz(I, J):
                tasks.flush(lambda key: key == (I, J))
                for p in range(8 * I, 8 * I + 8):
                    kvz_v[p] += lax.dot_general(vt.at[c, p][:, J * TH:(J + 1) * TH], phi[pl.ds(p * 128, 128), J * TH:(J + 1) * TH],
                                                NT, preferred_element_type=f32)
            pend = []

            def after(n, i):
                while pend:
                    kvz(*pend.pop(0))
                pend.extend(comp[n])
            pmatmul(SK, c, ordB, SMR, softmax_rows, tasks, after=after, bounce=via)
            if qpos == 0:
                prep_w_quarter(0, SQ, c, c)
            while pend:
                kvz(*pend.pop(0))
            prep_wo(c)
            return carry

        rr = lax.broadcasted_iota(jnp.int32, (80, 128), 0)
        cc = lax.broadcasted_iota(jnp.int32, (80, 128), 1)
        row_head = jnp.where(rr < 64, rr // 32, (rr - 64) // 8)
        mk = row_head == ((cc % 2) if pair else (cc // 64))

        def bodyC(c, carry):
            tasks = mk_tasks(SQ, 1)

            def nd_block(I, J):
                tasks.flush(lambda key: key == (I, J))
                t0 = J * TH
                for p in range(8 * I, 8 * I + 8):
                    kvm = jnp.where(mk, kvz_v[p], 0.0).astype(bf16)
                    nd = jnp.dot(kvm, phi[pl.ds(p * 128, 128), pl.ds(t0, TH)], preferred_element_type=f32)
                    rd = recip(nd[64:80] + 1e-6)
                    for hl in range(2):
                        rrep = jnp.concatenate([rd[hl * 8:hl * 8 + 8]] * 4, axis=0)
                        o32_v[pl.ds(p * 64 + hl * 32, 32), pl.ds(t0, TH)] = nd[hl * 32:hl * 32 + 32] * rrep

            def set_as(which):
                for r0 in range(0, DH, RB):
                    q = lambda T, K: o32_v[K * DH + r0:K * DH + r0 + RB, T * TH:(T + 1) * TH]
                    for i in which:
                        ot.at[i - 1][pl.ds(r0, RB), :] = lincomb([(sg, q(*k)) for sg, k in A_OPS[i]]).astype(bf16)

            def mo_(i):
                return jnp.dot(ot.at[i - 1][...].T, wos.at[i - 1][...], preferred_element_type=f32)

            def put_out(n, T, Cc):
                for q in range(0, TH, RB):
                    out_v[pl.ds(mo(c * TS + T * TH + q, RB), RB), Cc * DH:(Cc + 1) * DH] = \
                        lincomb([(sg, n[k][q:q + RB]) for sg, k in C_OPS[(T, Cc)]]).astype(bf16)

            assert tuple(ordC) == (5, 3, 1, 4, 7, 2, 6)

            def after(n, i):
                if n == 2:
                    nd_block(0, 1)
                elif n == 5:
                    nd_block(0, 0)
                    set_as([3, 6])
                elif n == 6:
                    nd_block(1, 0)
                    set_as([5])
            pmatmul(SQ, c, ordC, SMR, softmax_rows, tasks, after=after, bounce=via)
            n = {}
            n[3] = mo_(3)
            nd_block(1, 1)
            set_as([1, 2, 4, 7])
            n[6] = mo_(6)
            n[5] = mo_(5)
            put_out(n, 0, 1)
            cp_out(c, 0).start()
            n[1] = mo_(1)
            n[2] = mo_(2)
            put_out(n, 1, 1)
            n[4] = mo_(4)
            put_out(n, 1, 0)
            cp_out(c, 1).start()
            n[7] = mo_(7)
            put_out(n, 0, 0)
            cp_out(c, 2).start()
            return carry

        def run(body):
            lax.fori_loop(0, NC, body, 0)

        with sc("LA"):
            run(bodyA)
        with sc("mid"):
            cp_phi.wait()
            cp_w(1).wait()
            cp_w(0).wait()
            cp_wo.wait()
            build_bd()
            flag_s[0] = 0
            dz = flag_s[0]
            if qpos == 1:
                pass
            for part in range(4):
                prep_w_quarter(1, SK, part, dz + part)
                if qpos == 1:
                    prep_w_quarter(0, SQ, part, dz + part + 1)
        with sc("LB"):
            run(bodyB)
        with sc("LC"):
            run(bodyC)
        with sc("tail"):
            for c in range(NC):
                for k in range(3):
                    cp_out(c, k).wait()

    def wshape(l):
        return (7, DH // 2, DH) if l == 1 else (49, DQ // 2, DQ)

    def call(x, wqkv, w_phi, wo):
        x2 = x.reshape(S, D)
        wp = w_phi.reshape(H * Dh, Dh)
        out = pl.pallas_call(
            kernel,
            out_shape=jax.ShapeDtypeStruct((S, D), bf16),
            in_specs=[pl.BlockSpec(memory_space=pl.ANY)] * 4,
            out_specs=pl.BlockSpec(memory_space=pl.ANY),
            scratch_shapes=[
                pltpu.VMEM((S, D), bf16),
                pltpu.VMEM((D, 3 * D), bf16),
                pltpu.VMEM((D, D), bf16),
                pltpu.VMEM((H * Dh, Dh), bf16),
                pltpu.VMEM((S, D), bf16),
                pltpu.VMEM(wshape(lk), u32),
                pltpu.VMEM(wshape(lv), u32),
                pltpu.VMEM(wshape(lq), u32),
                pltpu.VMEM((NC, 7, TH // 2, DH) if X1 else (1, 7, 8, DH), u32),
                pltpu.VMEM((NC, 49, TQ // 2, DQ) if X2 else (1, 49, 8, DQ), u32),
                pltpu.VMEM((7, DH // 2, DH), u32),
                pltpu.VMEM((64, 1024), u32),
                pltpu.VMEM((NC, NP, 40, TS), u32),
                pltpu.VMEM((D, TS), u32),
                pltpu.VMEM((7, DH // 2, TH), u32),
                pltpu.VMEM((NP, 80, 128), f32),
                pltpu.VMEM((D, TS), f32),
                pltpu.VMEM((2, D, TS), f32),
                pltpu.VMEM((2, 256, 512), u32),
                pltpu.SMEM((8,), jnp.int32),
                pltpu.SemaphoreType.DMA((NC,)),
                pltpu.SemaphoreType.DMA((8,)),
                pltpu.SemaphoreType.DMA((3,)),
                pltpu.SemaphoreType.DMA((2,)),
                pltpu.SemaphoreType.DMA((NC, 3)),
            ],
            compiler_params=pltpu.CompilerParams(vmem_limit_bytes=110 * 1024 * 1024, flags=flags, disable_bounds_checks=nobc),
        )(x2, wqkv, wp, wo)
        return out.reshape(1, S, D)

    return call


_CALL = make_kernel(fstage=0, qpos=1)


@jax.jit
def pallas_standalone__linear_kernel_hedgehog__prompt_kernel(
    x: jax.Array,
    wqkv: jax.Array,
    w_phi: jax.Array,
    wo: jax.Array,
):
    return _CALL(x, wqkv, w_phi, wo)
```

```python
import jax
import jax.numpy as jnp
from jax import lax
from jax.experimental import pallas as pl
from jax.experimental.pallas import tpu as pltpu

LOG2E = 1.4426950408889634
NT = (((1,), (1,)), ((), ()))
f32, bf16, u32 = jnp.float32, jnp.bfloat16, jnp.uint32

S, D, H, Dh = 2048, 1024, 32, 32
TS = 512
NC, NP = S // TS, H // 2
TH, TQ, DH, DQ = TS // 2, TS // 4, D // 2, D // 4
RB = 16

A_OPS = {1: [(1, (0, 0)), (1, (1, 1))], 2: [(1, (1, 0)), (1, (1, 1))], 3: [(1, (0, 0))], 4: [(1, (1, 1))],
         5: [(1, (0, 0)), (1, (0, 1))], 6: [(1, (1, 0)), (-1, (0, 0))], 7: [(1, (0, 1)), (-1, (1, 1))]}
B_OPS = {1: [(1, (0, 0)), (1, (1, 1))], 2: [(1, (0, 0))], 3: [(1, (0, 1)), (-1, (1, 1))],
         4: [(1, (1, 0)), (-1, (0, 0))], 5: [(1, (1, 1))], 6: [(1, (0, 0)), (1, (0, 1))],
         7: [(1, (1, 0)), (1, (1, 1))]}
C_OPS = {(0, 0): [(1, 1), (1, 4), (-1, 5), (1, 7)], (0, 1): [(1, 3), (1, 5)],
         (1, 0): [(1, 2), (1, 4)], (1, 1): [(1, 1), (-1, 2), (1, 3), (1, 6)]}
ORD_EVEN = (5, 3, 2, 4, 1, 7, 6)
ORD_EARLY = (5, 3, 1, 4, 7, 2, 6)
ORD_OUT = (3, 6, 5, 1, 2, 4, 7)
WO_SLOTS = tuple(list(range(0, 8)) + list(range(14, 22)) + list(range(28, 40)))


def _al(v, m):
    return v if isinstance(v, int) else pl.multiple_of(v, m)


def _ds(start, size, m=None):
    return pl.ds(_al(start, m or size), size)


def _lin(terms):
    acc = terms[0][1]
    for sg, v in terms[1:]:
        acc = acc + v if sg > 0 else acc - v
    return acc


def _done(order):
    seen, out = set(), []
    for i in order:
        seen.add(i)
        out.append([q for q, t in C_OPS.items() if i in [k for _, k in t] and all(k in seen for _, k in t)])
    return out


def _inner_ops(table, i, blk):
    sub = {(a, b): _lin([(sg, blk(2 * k[0] + a, 2 * k[1] + b)) for sg, k in table[i]])
           for a in range(2) for b in range(2)}
    return {j: _lin([(sg, sub[k]) for sg, k in t]) for j, t in table.items()}


def _slot(i, j):
    return (i - 1) * 7 + j - 1


def _recip(x):
    return pltpu.reciprocal(x, approx=False, full_range=False)


def _allred(op, vs):
    while len(vs) > 1:
        vs = [op(vs[i], vs[i + 1]) for i in range(0, len(vs), 2)]
    v = op(vs[0], pltpu.roll(vs[0], 4, 0))
    return op(v, pltpu.roll(v, 2, 0))


def _kernel(x_hbm, w_hbm, wphi_hbm, wo_hbm, o_hbm,
            x_v, w_v, wphi_v, out_v, wk_u, wv_u, wq_u, xs_u, wos_u, bd_u, vt_u, phi_u, ot_u,
            kvz_v, o32_v, pbuf_v, sem_x, sem_wv, sem_w, sem_small, sem_o):
    wk, wv, wq, xs, wos, bd, vt, phi, ot = (
        r.bitcast(bf16) for r in (wk_u, wv_u, wq_u, xs_u, wos_u, bd_u, vt_u, phi_u, ot_u))

    def cp_x(c):
        return pltpu.make_async_copy(x_hbm.at[_ds(c * TS, TS), :], x_v.at[_ds(c * TS, TS), :], sem_x.at[c])

    def cp_wv(j):
        idx = (pl.ds(j * 128, 128), pl.ds(2 * D, D))
        return pltpu.make_async_copy(w_hbm.at[idx], w_v.at[idx], sem_wv.at[j])

    def cp_w(t):
        return pltpu.make_async_copy(w_hbm.at[:, pl.ds(t * D, D)], w_v.at[:, pl.ds(t * D, D)], sem_w.at[t])

    cp_phi = pltpu.make_async_copy(wphi_hbm, wphi_v, sem_small.at[0])
    cp_wo = pltpu.make_async_copy(wo_hbm, w_v.at[:, pl.ds(3 * D, D)], sem_small.at[1])

    def cp_out(c, k):
        r0, c0, nc = ((0, DH, DH), (TH, 0, D), (0, 0, DH))[k]
        idx = (_ds(c * TS + r0, TH), pl.ds(c0, nc))
        return pltpu.make_async_copy(out_v.at[idx], o_hbm.at[idx], sem_o.at[c, k])

    batches = ((0, 2, 4, 6), (1, 3, 5, 7))
    for b in batches:
        for j in b:
            cp_wv(j).start()
    cp_x(0).start()

    for c in range(NC):
        for p in range(NP):
            vt.at[c, p][64:80, :] = jnp.ones((16, TS), bf16)
    kvz_v[...] = jnp.zeros(kvz_v.shape, f32)

    def build_bd():
        r = lax.broadcasted_iota(jnp.int32, (128, 128), 0)
        cc = lax.broadcasted_iota(jnp.int32, (128, 128), 1)
        r2 = lax.broadcasted_iota(jnp.int32, (128, Dh), 0)
        perm = (((r2 % 64) // 8) * 4 + (r2 % 8) // 2 == lax.broadcasted_iota(jnp.int32, (128, Dh), 1)).astype(bf16)
        mask = ((r // 64) * 2 + r % 2) == (cc // 32)
        for g in range(8):
            t = lax.dot_general(perm, wphi_v[pl.ds(g * 128, 128), :], NT, preferred_element_type=f32)
            bd[:, pl.ds(g * 128, 128)] = jnp.where(mask, t, 0.0).astype(bf16)

    def w_tile(t, g, j):
        blk = w_v[pl.ds(j * 128, 128), pl.ds(t * D + g * 128, 128)]
        if t == 2:
            return blk.T
        res = lax.dot_general(bd[:, pl.ds(g * 128, 128)], blk, NT, preferred_element_type=f32)
        return (res * LOG2E).astype(bf16)

    def prep_w(t, dst, u, w):
        q = {(R, K): w_tile(t, 2 * R + u, 2 * K + w) for R in range(4) for K in range(4)}
        for r0 in range(0, 128, RB):
            sl = {k: v[r0:r0 + RB].astype(f32) for k, v in q.items()}
            for i in A_OPS:
                for j, v in _inner_ops(A_OPS, i, lambda R, K: sl[(R, K)]).items():
                    dst.at[_slot(i, j)][pl.ds(u * 128 + r0, RB), pl.ds(w * 128, 128)] = v.astype(bf16)

    def prep_x(c, i):
        for r0 in range(0, TQ, RB):
            def blk(K, J):
                return x_v[_ds(c * TS + J * TQ + r0, RB), K * DQ:(K + 1) * DQ].astype(f32)
            o = _inner_ops(B_OPS, i, blk)
            for j in ORD_EARLY:
                xs.at[c, _slot(i, j)][pl.ds(r0, RB), :] = o[j].astype(bf16)

    def prep_wo_piece(part, n, behind):
        r0, i = (n // 7) * RB, n % 7 + 1
        z = (pltpu.bitcast(behind, u32) >> 31) >> 1
        z = jnp.concatenate([z, z], axis=1)

        def blk(K, J):
            v = w_v[_ds(K * DQ + part * 64 + r0, RB), pl.ds(3 * D + J * DQ, DQ)]
            return pltpu.bitcast(pltpu.bitcast(v, u32) | z, bf16).astype(f32)
        for j, v in _inner_ops(B_OPS, i, blk).items():
            wos.at[_slot(i, j)][_ds(part * 64 + r0, RB), :] = v.astype(bf16)

    def softmax_pair(r0, t0, p):
        n = p.shape[1]
        ps = [p[t * 8:(t + 1) * 8] for t in range(8)]
        mx = _allred(jnp.maximum, ps)
        mn = _allred(jnp.minimum, ps)
        e1 = [jnp.exp2(v - mx) for v in ps]
        e2 = [jnp.exp2(mn - v) for v in ps]
        r1 = _recip(_allred(jnp.add, e1))
        r2 = _recip(_allred(jnp.add, e2))
        for es, r, off in ((e1, r1, 0), (e2, r2, 64)):
            for t in range(0, 8, 2):
                phi[pl.ds(2 * r0 + off + t * 8, 16), pl.ds(t0, n)] = \
                    jnp.concatenate([es[t] * r, es[t + 1] * r], axis=0).astype(bf16)

    def strassen(dot, rows, order, order_in, SL, consume, after=None, each=None):
        M = {}
        for n, (i, done) in enumerate(zip(order, _done(order))):
            m = {}
            for nj, (j, done_in) in enumerate(zip(order_in, _done(order_in))):
                m[j] = dot(_slot(i, j))
                if each:
                    each(n * 7 + nj, m[j])
                for (a, b) in done_in:
                    for r0 in range(0, rows, SL):
                        M[(i, a, b, r0)] = _lin([(sg, m[k][r0:r0 + SL]) for sg, k in C_OPS[(a, b)]])
                        for (I, J) in done:
                            consume((2 * I + a) * rows + r0, 2 * J + b,
                                    _lin([(sg, M[(k, a, b, r0)]) for sg, k in C_OPS[(I, J)]]))
            if after:
                after(n)

    def proj(w, c, order, order_in, SL, consume, **kw):
        strassen(lambda k: lax.dot_general(w.at[k][...], xs.at[c, k][...], NT, preferred_element_type=f32),
                 DQ, order, order_in, SL, lambda r0, tq, v: consume(r0, tq * TQ, v), **kw)

    for n, b in enumerate(batches):
        for j in b:
            cp_wv(j).wait()
        if n == 0:
            cp_phi.start()
            cp_w(1).start()
        for u in range(2):
            prep_w(2, wv, u, n)

    def body_v(c, carry):
        cp_x(c).wait()

        @pl.when(c + 1 < NC)
        def _():
            cp_x(c + 1).start()

        @pl.when(c == 1)
        def _():
            cp_w(0).start()

        @pl.when(c == 2)
        def _():
            cp_wo.start()
        for i in ORD_EVEN:
            prep_x(c, i)

        def put(r0, t0, v):
            vt.at[c, r0 // 64][pl.ds(r0 % 64, RB), pl.ds(t0, TQ)] = v.astype(bf16)
        proj(wv, c, ORD_EVEN, ORD_EARLY, RB, put)
        return carry

    lax.fori_loop(0, NC, body_v, 0)

    cp_phi.wait()
    cp_w(1).wait()
    cp_w(0).wait()
    cp_wo.wait()
    build_bd()
    for part in range(4):
        prep_w(1, wk, part // 2, part % 2)
        prep_w(0, wq, part // 2, part % 2)

    def body_k(c, carry):
        comp = _done(ORD_EVEN)

        def kvz(quads):
            for (I, J) in quads:
                for p in range(8 * I, 8 * I + 8):
                    kvz_v[p] += lax.dot_general(vt.at[c, p][:, J * TH:(J + 1) * TH],
                                                phi[pl.ds(p * 128, 128), J * TH:(J + 1) * TH],
                                                NT, preferred_element_type=f32)

        def each(n, m):
            if n in WO_SLOTS:
                prep_wo_piece(c, WO_SLOTS.index(n), m[DQ - 8:DQ])
        proj(wk, c, ORD_EVEN, ORD_EVEN, 64, softmax_pair,
             after=lambda n: kvz(comp[n - 1]) if n else None, each=each)
        kvz(comp[-1])
        return carry

    lax.fori_loop(0, NC, body_k, 0)

    rr = lax.broadcasted_iota(jnp.int32, (80, 128), 0)
    same_head = jnp.where(rr < 64, rr // 32, (rr - 64) // 8) == lax.broadcasted_iota(jnp.int32, (80, 128), 1) % 2

    def body_q(c, carry):
        pst, pld = pbuf_v.at[lax.rem(c, 2)], pbuf_v.at[c & 1]

        def via_vmem(r0, t0, v):
            pst[pl.ds(r0, 64), pl.ds(t0, TQ)] = v
            softmax_pair(r0, t0, pld[pl.ds(r0, 64), pl.ds(t0, TQ)])

        def nd(I, J):
            for p in range(8 * I, 8 * I + 8):
                kvm = jnp.where(same_head, kvz_v[p], 0.0).astype(bf16)
                r = jnp.dot(kvm, phi[pl.ds(p * 128, 128), pl.ds(J * TH, TH)], preferred_element_type=f32)
                rd = _recip(r[64:80] + 1e-6)
                for hl in range(2):
                    rep = jnp.concatenate([rd[hl * 8:hl * 8 + 8]] * 4, axis=0)
                    o32_v[pl.ds(p * 64 + hl * 32, 32), pl.ds(J * TH, TH)] = r[hl * 32:hl * 32 + 32] * rep

        def set_a(which):
            for i in which:
                for r0 in range(0, DQ, RB):
                    o = _inner_ops(A_OPS, i, lambda T, K: o32_v[pl.ds(K * DQ + r0, RB), pl.ds(T * TQ, TQ)])
                    for j, v in o.items():
                        ot.at[_slot(i, j)][pl.ds(r0, RB), 0:TQ] = v.astype(bf16)

        def after_q(n):
            if n == 2:
                nd(0, 1)
            elif n == 5:
                nd(0, 0)
                set_a([3, 6])
            elif n == 6:
                nd(1, 0)
                set_a([5])
        proj(wq, c, ORD_EARLY, ORD_EARLY, 64, via_vmem, after=after_q)

        def put_out(r0, cq, v):
            out_v[_ds(c * TS + r0, RB), pl.ds(cq * DQ, DQ)] = v.astype(bf16)

        def after_o(n):
            if n == 0:
                nd(1, 1)
                set_a([1, 2, 4, 7])
            elif n in (2, 5, 6):
                cp_out(c, {2: 0, 5: 1, 6: 2}[n]).start()
        strassen(lambda k: jnp.dot(ot.at[k][:, 0:TQ].T, wos.at[k][...], preferred_element_type=f32),
                 TQ, ORD_OUT, ORD_EARLY, RB, put_out, after=after_o)
        return carry

    lax.fori_loop(0, NC, body_q, 0)
    for c in range(NC):
        for k in range(3):
            cp_out(c, k).wait()


@jax.jit
def pallas_standalone__linear_kernel_hedgehog__prompt_kernel(x, wqkv, w_phi, wo):
    ops = pltpu.VMEM((49, DQ // 2, DQ), u32)
    out = pl.pallas_call(
        _kernel,
        out_shape=jax.ShapeDtypeStruct((S, D), bf16),
        in_specs=[pl.BlockSpec(memory_space=pl.ANY)] * 4,
        out_specs=pl.BlockSpec(memory_space=pl.ANY),
        scratch_shapes=[
            pltpu.VMEM((S, D), bf16),
            pltpu.VMEM((D, 4 * D), bf16),
            pltpu.VMEM((H * Dh, Dh), bf16),
            pltpu.VMEM((S, D), bf16),
            ops, ops, ops,
            pltpu.VMEM((NC, 49, TQ // 2, DQ), u32),
            ops,
            pltpu.VMEM((64, D), u32),
            pltpu.VMEM((NC, NP, 40, TS), u32),
            pltpu.VMEM((D, TS), u32),
            pltpu.VMEM((49, DQ // 2, 2 * TQ), u32),
            pltpu.VMEM((NP, 80, 128), f32),
            pltpu.VMEM((D, TS), f32),
            pltpu.VMEM((2, D, TS), f32),
            pltpu.SemaphoreType.DMA((NC,)),
            pltpu.SemaphoreType.DMA((8,)),
            pltpu.SemaphoreType.DMA((3,)),
            pltpu.SemaphoreType.DMA((2,)),
            pltpu.SemaphoreType.DMA((NC, 3)),
        ],
        compiler_params=pltpu.CompilerParams(vmem_limit_bytes=110 * 1024 * 1024, disable_bounds_checks=True),
    )(x.reshape(S, D), wqkv, w_phi.reshape(H * Dh, Dh), wo)
    return out.reshape(1, S, D)
```
